```python
import jax
import jax.numpy as jnp

def _softmax(x, axis=-1):
    return jax.nn.softmax(x, axis=axis)
def _gelu(x):
    return jax.nn.gelu(x, approximate=True)
def _silu(x):
    return jax.nn.silu(x)
def _sigmoid(x):
    return jax.nn.sigmoid(x)
def _layernorm(x, axis=-1, eps=1e-5):
    m = jnp.mean(x, axis=axis, keepdims=True)
    v = jnp.var(x, axis=axis, keepdims=True)
    return (x - m) / jnp.sqrt(v + eps)
def _scatter_add(tgt, idx, src, axis=0):
    return tgt.at[idx].add(src)
def _segment_sum(src, seg, n):
    return jax.ops.segment_sum(src, seg, n)
class _Rng:
    def __init__(self, key):
        self._k = key
    def _next(self):
        self._k, sub = jax.random.split(self._k)
        return sub
    def normal(self, shape):
        return jax.random.normal(self._next(), shape, dtype=jnp.bfloat16)
    def randint(self, lo, hi, shape):
        return jax.random.randint(self._next(), shape, lo, hi, dtype=jnp.int32)
    def uniform(self, shape, lo=0.0, hi=1.0):
        return jax.random.uniform(self._next(), shape, jnp.bfloat16, lo, hi)
    def permutation(self, n):
        return jax.random.permutation(self._next(), n)


kernel_name = 'sequential_preLN__grouped_kv_mqa__glu_gated_swiglu__prompt'

def _fwd_setup_inputs():
    _rng = _Rng(jax.random.key(int.from_bytes(__import__("os").urandom(4), "little")))
    _w = (lambda a: (lambda t: t.astype(jnp.bfloat16) if jnp.issubdtype(t.dtype, jnp.floating) else t)(jnp.asarray(a)))
    def _A_setup():
        B, S, D, H = 1, 2048, 512, 32
        Dh = D // H
        return {
            "x": _w((lambda *s: _rng.normal(s) * 0.05)(B, S, D)),
            "wq": _w((lambda *s: _rng.normal(s) * 0.05)(D, H * Dh)),
            "wk": _w((lambda *s: _rng.normal(s) * 0.05)(D, Dh)),
            "wv": _w((lambda *s: _rng.normal(s) * 0.05)(D, Dh)),
            "wo": _w((lambda *s: _rng.normal(s) * 0.05)(H * Dh, D)),
        }
    _A_in = _A_setup()

    def _B_setup():
        B, S, D, F = 1, 2048, 512, 1376
        return {
            "x": _w((lambda *s: _rng.normal(s) * 0.05)(B, S, D)),
            "w1": _w((lambda *s: _rng.normal(s) * 0.05)(D, F) * (2.0 / D) ** 0.5),
            "w3": _w((lambda *s: _rng.normal(s) * 0.05)(D, F) * (2.0 / D) ** 0.5),
            "w2": _w((lambda *s: _rng.normal(s) * 0.05)(F, D) * (2.0 / F) ** 0.5),
        }
    _B_in = _B_setup()

    return {
        "A_x": _A_in["x"],
        "A_wq": _A_in["wq"],
        "A_wk": _A_in["wk"],
        "A_wv": _A_in["wv"],
        "A_wo": _A_in["wo"],
        "B_x": _B_in["x"],
        "B_w1": _B_in["w1"],
        "B_w3": _B_in["w3"],
        "B_w2": _B_in["w2"],
    }

def _fwd_reference(A_x, A_wq, A_wk, A_wv, A_wo, B_x, B_w1, B_w3, B_w2):
    def _A_ref(x, wq, wk, wv, wo):
        B, S, D = x.shape
        H = 32
        Dh = D // H
        q = (lambda x, *d: x.transpose(*d))((x @ wq).reshape(B, S, H, Dh), 0, 2, 1, 3)
        k = x @ wk
        v = x @ wv
        scores = jnp.einsum("bhqd,bkd->bhqk", q, k) * (Dh ** -0.5)
        p = _softmax(scores, axis=-1)
        o = jnp.einsum("bhqk,bkd->bhqd", p, v)
        return (lambda x, *d: x.transpose(*d))(o, 0, 2, 1, 3).reshape(B, S, H * Dh) @ wo

    def _B_ref(x, w1, w3, w2):
        gate = jnp.einsum("bsd,df->bsf", x, w1)
        up = jnp.einsum("bsd,df->bsf", x, w3)
        h = _silu(gate) * up
        out = jnp.einsum("bsf,fd->bsd", h, w2)
        return out

    x = A_x
    h = x + _A_ref(_layernorm(x, axis=-1), A_wq, A_wk, A_wv, A_wo)
    h2 = h + _B_ref(_layernorm(h, axis=-1), B_w1, B_w3, B_w2)
    return h2


def setup_inputs():
    _inp = _fwd_setup_inputs()
    _gk = jax.random.fold_in(jax.random.key(int.from_bytes(__import__("os").urandom(4), "little")), 2**31 - 1)
    _shapes = [[1, 2048, 512]]
    _dtypes = ['bfloat16']
    _gks = jax.random.split(_gk, len(_shapes))
    _gs = [jax.random.normal(k, s, dtype=jnp.dtype(d)) * 0.05 for k, s, d in zip(_gks, _shapes, _dtypes)]
    _inp["grad_out"] = _gs[0]
    return _inp

def reference(A_x, A_wq, A_wk, A_wv, A_wo, B_w1, B_w3, B_w2, B_x, grad_out):
    _const = dict(B_x=B_x)
    def _f(*_d):
        return _fwd_reference(**{'A_x': _d[0], 'A_wq': _d[1], 'A_wk': _d[2], 'A_wv': _d[3], 'A_wo': _d[4], 'B_w1': _d[5], 'B_w3': _d[6], 'B_w2': _d[7], **_const})
    _out, _vjp = jax.vjp(_f, A_x, A_wq, A_wk, A_wv, A_wo, B_w1, B_w3, B_w2)
    _grads = _vjp(grad_out)
    _out0 = jnp.asarray(_out)
    return (_out0, *[jnp.asarray(_g) for _g in _grads])
```

```python
import jax
import jax.numpy as jnp
from jax import lax
import jax.experimental.pallas as pl
import jax.experimental.pallas.tpu as pltpu

S = 2048
D = 512
H = 32
DH = 16
F = 1376
BQ = 256
NB = S // BQ
EPS = 1e-5
SCALE = DH ** -0.5

f32 = jnp.float32
bf16 = jnp.bfloat16


def _ln(x):
    mu = jnp.mean(x, axis=-1, keepdims=True)
    xc = x - mu
    var = jnp.mean(xc * xc, axis=-1, keepdims=True)
    rstd = lax.rsqrt(var + EPS)
    return xc * rstd, rstd


def _ln_bwd(dy, xhat, rstd):
    m1 = jnp.mean(dy, axis=-1, keepdims=True)
    m2 = jnp.mean(dy * xhat, axis=-1, keepdims=True)
    return rstd * (dy - m1 - xhat * m2)


def _nn(a, b):
    return jnp.dot(a, b, preferred_element_type=f32)


def _nt(a, b):
    return lax.dot_general(a, b, (((1,), (1,)), ((), ())), preferred_element_type=f32)


def _tn(a, b):
    return lax.dot_general(a, b, (((0,), (0,)), ((), ())), preferred_element_type=f32)


def _kernel(x_ref, wq_ref, wk_ref, wv_ref, wo_ref, w1_ref, w3_ref, w2_ref, g_ref,
            out_ref, dx_ref, dwq_ref, dwk_ref, dwv_ref, dwo_ref, dw1_ref, dw3_ref, dw2_ref,
            ln1_s, k_s, v_s, kt_s, vt_s, e_s, linv_s, qt_s, ot_s, dot_s, dqt_s,
            dk_acc, dv_acc, dh_s, dl1_s, dwqt_acc, dwo_acc, dw1_acc, dw3_acc, dw2_acc):
    i = pl.program_id(0)

    @pl.when(i == 0)
    def _():
        def blk(b, c):
            r = pl.multiple_of(b * BQ, BQ)
            xf = x_ref[pl.ds(r, BQ), :].astype(f32)
            xhat, _ = _ln(xf)
            l1 = xhat.astype(bf16)
            ln1_s[pl.ds(r, BQ), :] = l1
            kk = _nn(l1, wk_ref[...])
            vv = _nn(l1, wv_ref[...])
            k_s[pl.ds(r, BQ), :] = kk.astype(bf16)
            v_s[pl.ds(r, BQ), :] = vv.astype(bf16)
            kt_s[:, pl.ds(r, BQ)] = kk.T.astype(bf16)
            vt_s[:, pl.ds(r, BQ)] = vv.T.astype(bf16)
            return c
        lax.fori_loop(0, NB, blk, 0)
        dk_acc[...] = jnp.zeros_like(dk_acc)
        dv_acc[...] = jnp.zeros_like(dv_acc)
        dwqt_acc[...] = jnp.zeros_like(dwqt_acc)
        dwo_acc[...] = jnp.zeros_like(dwo_acc)
        dw1_acc[...] = jnp.zeros_like(dw1_acc)
        dw3_acc[...] = jnp.zeros_like(dw3_acc)
        dw2_acc[...] = jnp.zeros_like(dw2_acc)

    r0 = pl.multiple_of(i * BQ, BQ)
    xf = x_ref[pl.ds(r0, BQ), :].astype(f32)
    l1 = ln1_s[pl.ds(r0, BQ), :]
    q = _nn(l1, wq_ref[...]) * SCALE
    qt_s[...] = q.T.astype(bf16)

    def fwd_head(h, c):
        r = pl.multiple_of(h * DH, DH)
        qt_h = qt_s[pl.ds(r, DH), :]
        st = _nn(k_s[...], qt_h)
        m = jnp.max(st, axis=0, keepdims=True)
        e = jnp.exp(st - m)
        l = jnp.sum(e, axis=0, keepdims=True)
        eb = e.astype(bf16)
        e_s[h] = eb
        linv = 1.0 / l
        linv_s[h] = linv
        ot = _nn(vt_s[...], eb)
        ot_s[pl.ds(r, DH), :] = ot * linv
        return c

    lax.fori_loop(0, H, fwd_head, 0)

    ot = ot_s[...]
    o_b = ot.T.astype(bf16)
    attn = _nn(o_b, wo_ref[...])
    h1 = xf + attn
    xhat2, rstd2 = _ln(h1)
    l2 = xhat2.astype(bf16)
    gate = _nn(l2, w1_ref[...])
    up = _nn(l2, w3_ref[...])
    sg = jax.nn.sigmoid(gate)
    silu = gate * sg
    hh = (silu * up).astype(bf16)
    y = h1 + _nn(hh, w2_ref[...])
    out_ref[...] = y.astype(bf16)

    g_b = g_ref[pl.ds(r0, BQ), :]
    dhh = _nt(g_b, w2_ref[...])
    dw2_acc[...] += _tn(hh, g_b)
    d_up = (dhh * silu).astype(bf16)
    d_gate = (dhh * up * (sg * (1.0 + gate * (1.0 - sg)))).astype(bf16)
    dl2 = _nt(d_gate, w1_ref[...]) + _nt(d_up, w3_ref[...])
    dw1_acc[...] += _tn(l2, d_gate)
    dw3_acc[...] += _tn(l2, d_up)
    dh = g_b.astype(f32) + _ln_bwd(dl2, xhat2, rstd2)
    dh_s[pl.ds(r0, BQ), :] = dh
    dh_b = dh.astype(bf16)

    dot_s[...] = _nt(wo_ref[...], dh_b)
    dwo_acc[...] += _nn(ot.astype(bf16), dh_b)

    def bwd_head(h, c):
        r = pl.multiple_of(h * DH, DH)
        linv = linv_s[h]
        dot_h = dot_s[pl.ds(r, DH), :] * linv
        ot_h = ot_s[pl.ds(r, DH), :]
        delta = jnp.sum(dot_h * ot_h, axis=0, keepdims=True)
        dob = dot_h.astype(bf16)
        dpt = _nn(v_s[...], dob)
        eb = e_s[h]
        dst = (eb.astype(f32) * (dpt - delta)).astype(bf16)
        dqt_s[pl.ds(r, DH), :] = _nn(kt_s[...], dst)
        qt_h = qt_s[pl.ds(r, DH), :]
        dk_acc[...] += _nt(dst, qt_h)
        dv_acc[...] += _nt(eb, dob)
        return c

    lax.fori_loop(0, H, bwd_head, 0)

    dqt = dqt_s[...] * SCALE
    dqt_b = dqt.astype(bf16)
    dq_b = dqt.T.astype(bf16)
    dl1_s[pl.ds(r0, BQ), :] = _nt(dq_b, wq_ref[...])
    dwqt_acc[...] += _nn(dqt_b, l1)

    @pl.when(i == NB - 1)
    def _():
        dkb = dk_acc[...].astype(bf16)
        dvb = dv_acc[...].astype(bf16)
        l1_all = ln1_s[...]
        dwk_ref[...] = _tn(l1_all, dkb).astype(bf16)
        dwv_ref[...] = _tn(l1_all, dvb).astype(bf16)

        def blk(b, c):
            r = pl.multiple_of(b * BQ, BQ)
            xb = x_ref[pl.ds(r, BQ), :].astype(f32)
            xhat, rstd = _ln(xb)
            dl1 = (dl1_s[pl.ds(r, BQ), :]
                   + _nt(dk_acc[pl.ds(r, BQ), :].astype(bf16), wk_ref[...])
                   + _nt(dv_acc[pl.ds(r, BQ), :].astype(bf16), wv_ref[...]))
            dxv = dh_s[pl.ds(r, BQ), :] + _ln_bwd(dl1, xhat, rstd)
            dx_ref[pl.ds(r, BQ), :] = dxv.astype(bf16)
            return c
        lax.fori_loop(0, NB, blk, 0)
        dwq_ref[...] = dwqt_acc[...].T.astype(bf16)
        dwo_ref[...] = dwo_acc[...].astype(bf16)
        dw1_ref[...] = dw1_acc[...].astype(bf16)
        dw3_ref[...] = dw3_acc[...].astype(bf16)
        dw2_ref[...] = dw2_acc[...].astype(bf16)


@jax.jit
def pallas_sequential_preLN__grouped_kv_mqa__glu_gated_swiglu__prompt_kernel(
    A_x: jax.Array,
    A_wq: jax.Array,
    A_wk: jax.Array,
    A_wv: jax.Array,
    A_wo: jax.Array,
    B_x: jax.Array,
    B_w1: jax.Array,
    B_w3: jax.Array,
    B_w2: jax.Array,
    grad_out: jax.Array,
):
    del B_x
    x2 = A_x.reshape(S, D)
    g2 = grad_out.reshape(S, D)

    def full(shape):
        return pl.BlockSpec(shape, lambda i: (0,) * len(shape))

    in_specs = [
        full((S, D)), full((D, D)), full((D, DH)), full((D, DH)), full((D, D)),
        full((D, F)), full((D, F)), full((F, D)), full((S, D)),
    ]
    out_specs = [
        pl.BlockSpec((BQ, D), lambda i: (i, 0)),
        full((S, D)), full((D, D)), full((D, DH)), full((D, DH)), full((D, D)),
        full((D, F)), full((D, F)), full((F, D)),
    ]
    out_shape = [
        jax.ShapeDtypeStruct((S, D), bf16),
        jax.ShapeDtypeStruct((S, D), bf16),
        jax.ShapeDtypeStruct((D, D), bf16),
        jax.ShapeDtypeStruct((D, DH), bf16),
        jax.ShapeDtypeStruct((D, DH), bf16),
        jax.ShapeDtypeStruct((D, D), bf16),
        jax.ShapeDtypeStruct((D, F), bf16),
        jax.ShapeDtypeStruct((D, F), bf16),
        jax.ShapeDtypeStruct((F, D), bf16),
    ]
    scratch_shapes = [
        pltpu.VMEM((S, D), bf16),
        pltpu.VMEM((S, DH), bf16),
        pltpu.VMEM((S, DH), bf16),
        pltpu.VMEM((DH, S), bf16),
        pltpu.VMEM((DH, S), bf16),
        pltpu.VMEM((H, S, BQ), bf16),
        pltpu.VMEM((H, 1, BQ), f32),
        pltpu.VMEM((D, BQ), bf16),
        pltpu.VMEM((D, BQ), f32),
        pltpu.VMEM((D, BQ), f32),
        pltpu.VMEM((D, BQ), f32),
        pltpu.VMEM((S, DH), f32),
        pltpu.VMEM((S, DH), f32),
        pltpu.VMEM((S, D), f32),
        pltpu.VMEM((S, D), f32),
        pltpu.VMEM((D, D), f32),
        pltpu.VMEM((D, D), f32),
        pltpu.VMEM((D, F), f32),
        pltpu.VMEM((D, F), f32),
        pltpu.VMEM((F, D), f32),
    ]
    outs = pl.pallas_call(
        _kernel,
        grid=(NB,),
        in_specs=in_specs,
        out_specs=out_specs,
        out_shape=out_shape,
        scratch_shapes=scratch_shapes,
        compiler_params=pltpu.CompilerParams(
            dimension_semantics=("arbitrary",),
            vmem_limit_bytes=112 * 1024 * 1024,
        ),
    )(x2, A_wq, A_wk, A_wv, A_wo, B_w1, B_w3, B_w2, g2)
    out, dx, dwq, dwk, dwv, dwo, dw1, dw3, dw2 = outs
    return (out.reshape(1, S, D), dx.reshape(1, S, D), dwq, dwk, dwv, dwo, dw1, dw3, dw2)
```

```python
import jax
import jax.numpy as jnp
from jax import lax
import jax.experimental.pallas as pl
import jax.experimental.pallas.tpu as pltpu

S = 2048
D = 512
H = 32
DH = 16
F = 1376
BQ = 256
NB = S // BQ
EPS = 1e-5
SCALE = DH ** -0.5
NSPLIT = 8
LOG2E = 1.4426950408889634
LN2 = 0.6931471805599453

f32 = jnp.float32
bf16 = jnp.bfloat16


def _ln(x):
    mu = jnp.mean(x, axis=-1, keepdims=True)
    xc = x - mu
    var = jnp.mean(xc * xc, axis=-1, keepdims=True)
    rstd = lax.rsqrt(var + EPS)
    return xc * rstd, rstd


def _ln_bwd(dy, xhat, rstd):
    m1 = jnp.mean(dy, axis=-1, keepdims=True)
    m2 = jnp.mean(dy * xhat, axis=-1, keepdims=True)
    return rstd * (dy - m1 - xhat * m2)


def _nn(a, b):
    return jnp.dot(a, b, preferred_element_type=f32)


def _nt(a, b):
    return lax.dot_general(a, b, (((1,), (1,)), ((), ())), preferred_element_type=f32)


def _tn(a, b):
    return lax.dot_general(a, b, (((0,), (0,)), ((), ())), preferred_element_type=f32)


def _kernel(x_ref, wq_ref, wk_ref, wv_ref, wo_ref, w1_ref, w3_ref, w2_ref, g_ref,
            out_ref, dx_ref, dwq_ref, dwk_ref, dwv_ref, dwo_ref, dw1_ref, dw3_ref, dw2_ref,
            ln1_s, k_s, v_s, kt_s, vt_s, e_s, linv_s, qt_s, ot_s, dot_s, dqt_s,
            dk_acc, dv_acc, dh_s, dl1_s, dwqt_acc, dwo_acc, dw1_acc, dw3_acc, dw2_acc, sa_s, sb_s, dob_s):
    i = pl.program_id(0)

    @pl.when(i == 0)
    def _():
        def blk(b, c):
            r = pl.multiple_of(b * BQ, BQ)
            xf = x_ref[pl.ds(r, BQ), :].astype(f32)
            xhat, _ = _ln(xf)
            l1 = xhat.astype(bf16)
            ln1_s[pl.ds(r, BQ), :] = l1
            kk = _nn(l1, wk_ref[...])
            vv = _nn(l1, wv_ref[...])
            k_s[pl.ds(r, BQ), :] = kk.astype(bf16)
            v_s[pl.ds(r, BQ), :] = vv.astype(bf16)
            kt_s[:, pl.ds(r, BQ)] = kk.T.astype(bf16)
            vt_s[:, pl.ds(r, BQ)] = vv.T.astype(bf16)
            return c
        lax.fori_loop(0, NB, blk, 0)
        dk_acc[...] = jnp.zeros_like(dk_acc)
        dv_acc[...] = jnp.zeros_like(dv_acc)
        dwqt_acc[...] = jnp.zeros_like(dwqt_acc)
        dwo_acc[...] = jnp.zeros_like(dwo_acc)
        dw1_acc[...] = jnp.zeros_like(dw1_acc)
        dw3_acc[...] = jnp.zeros_like(dw3_acc)
        dw2_acc[...] = jnp.zeros_like(dw2_acc)

    r0 = pl.multiple_of(i * BQ, BQ)
    xf = x_ref[pl.ds(r0, BQ), :].astype(f32)
    l1 = ln1_s[pl.ds(r0, BQ), :]
    q = _nn(l1, wq_ref[...]) * (SCALE * LOG2E)
    qt_s[...] = q.T.astype(bf16)

    def compute_s(h, dst):
        r = pl.multiple_of(h * DH, DH)
        qt_h = qt_s[pl.ds(r, DH), :]
        for c4 in range(NSPLIT):
            lo, hi = c4 * (S // NSPLIT), (c4 + 1) * (S // NSPLIT)
            dst[lo:hi, :] = _nn(k_s[lo:hi, :], qt_h)

    def softmax_o(h, src):
        r = pl.multiple_of(h * DH, DH)
        st = src[...]
        m = jnp.max(st, axis=0, keepdims=True)
        e = jnp.exp2(st - m)
        l = jnp.sum(e, axis=0, keepdims=True)
        eb = e.astype(bf16)
        e_s[h] = eb
        linv = 1.0 / l
        linv_s[h] = linv
        ot = _nn(vt_s[...], eb)
        ot_s[pl.ds(r, DH), :] = ot * linv

    compute_s(0, sa_s)

    def fwd_pair(j, c):
        h0 = 2 * j
        h1 = h0 + 1
        h2 = jnp.minimum(h0 + 2, H - 1)
        compute_s(h1, sb_s)
        softmax_o(h0, sa_s)
        compute_s(h2, sa_s)
        softmax_o(h1, sb_s)
        return c

    lax.fori_loop(0, H // 2, fwd_pair, 0)

    ot = ot_s[...]
    o_b = ot.T.astype(bf16)
    attn = _nn(o_b, wo_ref[...])
    h1 = xf + attn
    xhat2, rstd2 = _ln(h1)
    l2 = xhat2.astype(bf16)
    gate = _nn(l2, w1_ref[...])
    up = _nn(l2, w3_ref[...])
    sg = jax.nn.sigmoid(gate)
    silu = gate * sg
    hh = (silu * up).astype(bf16)
    y = h1 + _nn(hh, w2_ref[...])
    out_ref[...] = y.astype(bf16)

    g_b = g_ref[pl.ds(r0, BQ), :]
    dhh = _nt(g_b, w2_ref[...])
    dw2_acc[...] += _tn(hh, g_b)
    d_up = (dhh * silu).astype(bf16)
    d_gate = (dhh * up * (sg * (1.0 + gate * (1.0 - sg)))).astype(bf16)
    dl2 = _nt(d_gate, w1_ref[...]) + _nt(d_up, w3_ref[...])
    dw1_acc[...] += _tn(l2, d_gate)
    dw3_acc[...] += _tn(l2, d_up)
    dh = g_b.astype(f32) + _ln_bwd(dl2, xhat2, rstd2)
    dh_s[pl.ds(r0, BQ), :] = dh
    dh_b = dh.astype(bf16)

    dot_s[...] = _nt(wo_ref[...], dh_b)
    dwo_acc[...] += _nn(ot.astype(bf16), dh_b)

    def bwd_prep(h, dst_buf):
        r = pl.multiple_of(h * DH, DH)
        dot_h = dot_s[pl.ds(r, DH), :] * linv_s[h]
        dob = dot_h.astype(bf16)
        dob_s[pl.ds(r, DH), :] = dob
        for c4 in range(NSPLIT):
            lo, hi = c4 * (S // NSPLIT), (c4 + 1) * (S // NSPLIT)
            dst_buf[lo:hi, :] = _nn(v_s[lo:hi, :], dob)

    def bwd_fin(h, src_buf):
        r = pl.multiple_of(h * DH, DH)
        dot_h = dot_s[pl.ds(r, DH), :] * linv_s[h]
        ot_h = ot_s[pl.ds(r, DH), :]
        delta = jnp.sum(dot_h * ot_h, axis=0, keepdims=True)
        eb = e_s[h]
        dst = (eb.astype(f32) * (src_buf[...] - delta)).astype(bf16)
        dqt_s[pl.ds(r, DH), :] = _nn(kt_s[...], dst)
        qt_h = qt_s[pl.ds(r, DH), :]
        dk_acc[...] += _nt(qt_h, dst)
        dv_acc[...] += _nt(dob_s[pl.ds(r, DH), :], eb)

    bwd_prep(0, sa_s)

    def bwd_pair(j, c):
        h0 = 2 * j
        h1 = h0 + 1
        h2 = jnp.minimum(h0 + 2, H - 1)
        bwd_prep(h1, sb_s)
        bwd_fin(h0, sa_s)
        bwd_prep(h2, sa_s)
        bwd_fin(h1, sb_s)
        return c

    lax.fori_loop(0, H // 2, bwd_pair, 0)

    dqt = dqt_s[...] * SCALE
    dqt_b = dqt.astype(bf16)
    dq_b = dqt.T.astype(bf16)
    dl1_s[pl.ds(r0, BQ), :] = _nt(dq_b, wq_ref[...])
    dwqt_acc[...] += _nn(dqt_b, l1)

    @pl.when(i == NB - 1)
    def _():
        l1_all = ln1_s[...]
        dwk_ref[...] = _nn((dk_acc[...] * LN2).astype(bf16), l1_all).T.astype(bf16)
        dwv_ref[...] = _nn(dv_acc[...].astype(bf16), l1_all).T.astype(bf16)

        def blk(b, c):
            r = pl.multiple_of(b * BQ, BQ)
            xb = x_ref[pl.ds(r, BQ), :].astype(f32)
            xhat, rstd = _ln(xb)
            dl1 = (dl1_s[pl.ds(r, BQ), :]
                   + _nt((dk_acc[:, pl.ds(r, BQ)] * LN2).T.astype(bf16), wk_ref[...])
                   + _nt(dv_acc[:, pl.ds(r, BQ)].T.astype(bf16), wv_ref[...]))
            dxv = dh_s[pl.ds(r, BQ), :] + _ln_bwd(dl1, xhat, rstd)
            dx_ref[pl.ds(r, BQ), :] = dxv.astype(bf16)
            return c
        lax.fori_loop(0, NB, blk, 0)
        dwq_ref[...] = dwqt_acc[...].T.astype(bf16)
        dwo_ref[...] = dwo_acc[...].astype(bf16)
        dw1_ref[...] = dw1_acc[...].astype(bf16)
        dw3_ref[...] = dw3_acc[...].astype(bf16)
        dw2_ref[...] = dw2_acc[...].astype(bf16)


@jax.jit
def pallas_sequential_preLN__grouped_kv_mqa__glu_gated_swiglu__prompt_kernel(
    A_x: jax.Array,
    A_wq: jax.Array,
    A_wk: jax.Array,
    A_wv: jax.Array,
    A_wo: jax.Array,
    B_x: jax.Array,
    B_w1: jax.Array,
    B_w3: jax.Array,
    B_w2: jax.Array,
    grad_out: jax.Array,
):
    del B_x
    x2 = A_x.reshape(S, D)
    g2 = grad_out.reshape(S, D)

    def full(shape):
        return pl.BlockSpec(shape, lambda i: (0,) * len(shape))

    in_specs = [
        full((S, D)), full((D, D)), full((D, DH)), full((D, DH)), full((D, D)),
        full((D, F)), full((D, F)), full((F, D)), full((S, D)),
    ]
    out_specs = [
        pl.BlockSpec((BQ, D), lambda i: (i, 0)),
        full((S, D)), full((D, D)), full((D, DH)), full((D, DH)), full((D, D)),
        full((D, F)), full((D, F)), full((F, D)),
    ]
    out_shape = [
        jax.ShapeDtypeStruct((S, D), bf16),
        jax.ShapeDtypeStruct((S, D), bf16),
        jax.ShapeDtypeStruct((D, D), bf16),
        jax.ShapeDtypeStruct((D, DH), bf16),
        jax.ShapeDtypeStruct((D, DH), bf16),
        jax.ShapeDtypeStruct((D, D), bf16),
        jax.ShapeDtypeStruct((D, F), bf16),
        jax.ShapeDtypeStruct((D, F), bf16),
        jax.ShapeDtypeStruct((F, D), bf16),
    ]
    scratch_shapes = [
        pltpu.VMEM((S, D), bf16),
        pltpu.VMEM((S, DH), bf16),
        pltpu.VMEM((S, DH), bf16),
        pltpu.VMEM((DH, S), bf16),
        pltpu.VMEM((DH, S), bf16),
        pltpu.VMEM((H, S, BQ), bf16),
        pltpu.VMEM((H, 1, BQ), f32),
        pltpu.VMEM((D, BQ), bf16),
        pltpu.VMEM((D, BQ), f32),
        pltpu.VMEM((D, BQ), f32),
        pltpu.VMEM((D, BQ), f32),
        pltpu.VMEM((DH, S), f32),
        pltpu.VMEM((DH, S), f32),
        pltpu.VMEM((S, D), f32),
        pltpu.VMEM((S, D), f32),
        pltpu.VMEM((D, D), f32),
        pltpu.VMEM((D, D), f32),
        pltpu.VMEM((D, F), f32),
        pltpu.VMEM((D, F), f32),
        pltpu.VMEM((F, D), f32),
        pltpu.VMEM((S, BQ), f32),
        pltpu.VMEM((S, BQ), f32),
        pltpu.VMEM((D, BQ), bf16),
    ]
    outs = pl.pallas_call(
        _kernel,
        grid=(NB,),
        in_specs=in_specs,
        out_specs=out_specs,
        out_shape=out_shape,
        scratch_shapes=scratch_shapes,
        compiler_params=pltpu.CompilerParams(
            dimension_semantics=("arbitrary",),
            vmem_limit_bytes=112 * 1024 * 1024,
        ),
    )(x2, A_wq, A_wk, A_wv, A_wo, B_w1, B_w3, B_w2, g2)
    out, dx, dwq, dwk, dwv, dwo, dw1, dw3, dw2 = outs
    return (out.reshape(1, S, D), dx.reshape(1, S, D), dwq, dwk, dwv, dwo, dw1, dw3, dw2)
```
